```python
import jax
import jax.numpy as jnp

def _softmax(x, axis=-1):
    return jax.nn.softmax(x, axis=axis)
def _gelu(x):
    return jax.nn.gelu(x, approximate=True)
def _silu(x):
    return jax.nn.silu(x)
def _sigmoid(x):
    return jax.nn.sigmoid(x)
def _layernorm(x, axis=-1, eps=1e-5):
    m = jnp.mean(x, axis=axis, keepdims=True)
    v = jnp.var(x, axis=axis, keepdims=True)
    return (x - m) / jnp.sqrt(v + eps)
def _scatter_add(tgt, idx, src, axis=0):
    return tgt.at[idx].add(src)
def _segment_sum(src, seg, n):
    return jax.ops.segment_sum(src, seg, n)
class _Rng:
    def __init__(self, key):
        self._k = key
    def _next(self):
        self._k, sub = jax.random.split(self._k)
        return sub
    def normal(self, shape):
        return jax.random.normal(self._next(), shape, dtype=jnp.bfloat16)
    def randint(self, lo, hi, shape):
        return jax.random.randint(self._next(), shape, lo, hi, dtype=jnp.int32)
    def uniform(self, shape, lo=0.0, hi=1.0):
        return jax.random.uniform(self._next(), shape, jnp.bfloat16, lo, hi)
    def permutation(self, n):
        return jax.random.permutation(self._next(), n)


kernel_name = 'parallel_sum__sliding_block_cached__moe_arch_mod__decode'

def setup_inputs():
    _rng = _Rng(jax.random.key(int.from_bytes(__import__("os").urandom(4), "little")))
    _w = (lambda a: (lambda t: t.astype(jnp.bfloat16) if jnp.issubdtype(t.dtype, jnp.floating) else t)(jnp.asarray(a)))
    def _A_setup():
        B, Sq, D = 1, 1, 512
        Hq, Hkv, Sk, Dh = 32, 8, 65536, 128
        assert Hq % Hkv == 0, (Hq, Hkv)
        return {
            "x": _w((lambda *s: _rng.normal(s) * 0.05)(B, Sq, D)),
            "k_cache": _w((lambda *s: _rng.normal(s) * 0.05)(B, Hkv, Sk, Dh)),
            "v_cache": _w((lambda *s: _rng.normal(s) * 0.05)(B, Hkv, Sk, Dh)),
            "wq": _w((lambda *s: _rng.normal(s) * 0.05)(D, Hq * Dh) * (D ** -0.5)),
            "wo": _w((lambda *s: _rng.normal(s) * 0.05)(Hq * Dh, D) * ((Hq * Dh) ** -0.5)),
        }
    _A_in = _A_setup()

    def _B_setup():
        B, S, D, F, C = 1, 1, 512, 1792, 1
        return {
            "x": _w((lambda *s: _rng.normal(s) * 0.05)(B, S, D)),
            "w_r": _w((lambda *s: _rng.normal(s) * 0.05)(D)),
            "w_gate": _w((lambda *s: _rng.normal(s) * 0.05)(D, F)),
            "w_up": _w((lambda *s: _rng.normal(s) * 0.05)(D, F)),
            "w_down": _w((lambda *s: _rng.normal(s) * 0.05)(F, D)),
        }
    _B_in = _B_setup()

    return {
        "A_x": _A_in["x"],
        "A_k_cache": _A_in["k_cache"],
        "A_v_cache": _A_in["v_cache"],
        "A_wq": _A_in["wq"],
        "A_wo": _A_in["wo"],
        "B_x": _B_in["x"],
        "B_w_r": _B_in["w_r"],
        "B_w_gate": _B_in["w_gate"],
        "B_w_up": _B_in["w_up"],
        "B_w_down": _B_in["w_down"],
    }

def reference(A_x, A_k_cache, A_v_cache, A_wq, A_wo, B_x, B_w_r, B_w_gate, B_w_up, B_w_down):
    def _A_ref(x, k_cache, v_cache, wq, wo):
        B, Sq, D = x.shape
        Hq, Dh = 32, 128
        Hkv, Sk = k_cache.shape[1], k_cache.shape[2]
        W = min(4096, max(256, Sk // 4))
        rep = Hq // Hkv
        q = (lambda x, *d: x.transpose(*d))((x @ wq).reshape(B, Sq, Hq, Dh), 0, 2, 1, 3)
        k = jnp.repeat(k_cache[:, :, Sk - W:, :], rep, axis=1)
        v = jnp.repeat(v_cache[:, :, Sk - W:, :], rep, axis=1)
        scores = jnp.einsum("bhqd,bhkd->bhqk", q, k) * (Dh ** -0.5)
        p = _softmax(scores, axis=-1)
        o = jnp.einsum("bhqk,bhkd->bhqd", p, v)
        return (lambda x, *d: x.transpose(*d))(o, 0, 2, 1, 3).reshape(B, Sq, Hq * Dh) @ wo

    def _B_ref(x, w_r, w_gate, w_up, w_down):
        B, S, D = x.shape
        C = 1
        r = x @ w_r
        idx = jnp.argsort(-r, axis=-1)[:, :C]
        idx_e = jnp.repeat(idx.reshape(B, C, 1), D, axis=2)
        x_sel = jnp.take_along_axis(x, idx_e, axis=1)
        g = _silu(x_sel @ w_gate)
        u = x_sel @ w_up
        y = (g * u) @ w_down
        r_sel = _sigmoid(jnp.take_along_axis(r, idx, axis=1))
        y = y * r_sel.reshape(B, C, 1)
        b_off = (jnp.arange(B) * S).reshape(B, 1)
        flat_idx = (idx + b_off).reshape(B * C)
        zero = (x * 0.0).reshape(B * S, D)
        upd = _scatter_add(zero, flat_idx, y.reshape(B * C, D), axis=0)
        return x + upd.reshape(B, S, D)

    x = A_x
    xn = _layernorm(x, axis=-1)
    return x + _A_ref(xn, A_k_cache, A_v_cache, A_wq, A_wo) + _B_ref(xn, B_w_r, B_w_gate, B_w_up, B_w_down)
```

```python
import numpy as np

import jax
import jax.numpy as jnp
import jax.experimental.pallas as pl
import jax.experimental.pallas.tpu as pltpu

HQ, DH = 32, 128
EPS = 1e-5
WD_CHUNKS = (1024, 512, 128, 128)

f32, bf16 = jnp.float32, jnp.bfloat16


def _make_kernel(D, HKV, SK, W, F):
    rep = HQ // HKV
    gcols = rep * DH
    nwd = len(WD_CHUNKS)
    wd_off = [int(o) for o in np.cumsum((0,) + WD_CHUNKS)]
    assert wd_off[-1] == F
    S_X, S_WR, S_WQ, S_WG, S_WU, S_WD = range(6)
    S_K = S_WD + nwd
    S_V = S_K + HKV
    S_WO = S_V + HKV
    nsem = S_WO + HKV
    scale = np.float32(DH ** -0.5)

    def kernel(x_hbm, k_hbm, v_hbm, wq_hbm, wo_hbm, wr_hbm, wg_hbm, wu_hbm, wd_hbm, o_ref,
               xb, wrb, kb, vb, wqb, wob, wgb, wub, wdb, qs, sems):
        win = pl.ds(SK - W, W)
        cp = pltpu.make_async_copy
        x_cp = cp(x_hbm, xb, sems.at[S_X])
        wr_cp = cp(wr_hbm, wrb, sems.at[S_WR])
        wq_cp = cp(wq_hbm, wqb, sems.at[S_WQ])
        wg_cp = cp(wg_hbm, wgb, sems.at[S_WG])
        wu_cp = cp(wu_hbm, wub, sems.at[S_WU])

        def wd_cp(i):
            sl = pl.ds(wd_off[i], WD_CHUNKS[i])
            return cp(wd_hbm.at[sl, :], wdb.at[sl, :], sems.at[S_WD + i])

        def k_cp(g):
            return cp(k_hbm.at[0, g, win, :], kb.at[g], sems.at[S_K + g])

        def v_cp(g):
            return cp(v_hbm.at[0, g, win, :], vb.at[g], sems.at[S_V + g])

        def wo_cp(g):
            sl = pl.ds(pl.multiple_of(g * gcols, gcols), gcols)
            return cp(wo_hbm.at[sl, :], wob.at[sl, :], sems.at[S_WO + g])

        x_cp.start()
        wr_cp.start()
        wq_cp.start()
        wg_cp.start()
        wu_cp.start()

        def issue(g, c):
            k_cp(g).start()
            v_cp(g).start()
            wo_cp(g).start()
            return c

        jax.lax.fori_loop(0, HKV, issue, 0)
        for i in range(nwd):
            wd_cp(i).start()

        x_cp.wait()
        wr_cp.wait()
        x = xb[0].astype(f32)
        mu = jnp.mean(x, axis=-1, keepdims=True)
        xc = x - mu
        var = jnp.mean(xc * xc, axis=-1, keepdims=True)
        xn = (xc / jnp.sqrt(var + EPS)).astype(bf16).astype(f32)
        r = jnp.sum(xn * wrb[...].astype(f32).reshape(1, D), axis=-1, keepdims=True)
        r_sel = jax.nn.sigmoid(r.astype(bf16).astype(f32))
        xn8 = jnp.broadcast_to(xn, (8, D)).astype(bf16)

        row = jax.lax.broadcasted_iota(jnp.int32, (8, DH), 0)

        wq_cp.wait()
        for g in range(HKV):
            qc = jnp.dot(xn8, wqb[:, g * gcols:(g + 1) * gcols], preferred_element_type=f32)
            qg = qc[:, 0:DH]
            for j in range(1, rep):
                qg = jnp.where(row == j, qc[:, j * DH:(j + 1) * DH], qg)
            qs[g] = qg

        wg_cp.wait()
        gate = jnp.dot(xn8, wgb[...], preferred_element_type=f32).astype(bf16).astype(f32)
        wu_cp.wait()
        up = jnp.dot(xn8, wub[...], preferred_element_type=f32).astype(bf16).astype(f32)
        h = (jax.nn.silu(gate) * up).astype(bf16)

        def attn(g, acc):
            k_cp(g).wait()
            q = qs[g].astype(bf16)
            s = jax.lax.dot_general(q, kb[g], (((1,), (1,)), ((), ())), preferred_element_type=f32)
            m = jnp.max(s, axis=-1, keepdims=True)
            p = jnp.exp((s - m) * scale)
            l = jnp.sum(p, axis=-1, keepdims=True)
            v_cp(g).wait()
            o = jnp.dot(p.astype(bf16), vb[g], preferred_element_type=f32) / l
            o = o.astype(bf16).astype(f32)
            lhs = jnp.concatenate([jnp.where(row == j, o, 0.0) for j in range(rep)], axis=1).astype(bf16)
            wo_cp(g).wait()
            w = wob[pl.ds(pl.multiple_of(g * gcols, gcols), gcols), :]
            return acc + jnp.dot(lhs, w, preferred_element_type=f32)

        acc = jax.lax.fori_loop(0, HKV, attn, jnp.zeros((8, D), f32))
        base = x + jnp.sum(acc, axis=0, keepdims=True) + xn

        y = jnp.zeros((8, D), f32)
        for i in range(nwd):
            wd_cp(i).wait()
            lo, hi = wd_off[i], wd_off[i + 1]
            y = y + jnp.dot(h[:, lo:hi], wdb[lo:hi, :], preferred_element_type=f32)
        o_ref[0] = (base + y[0:1] * r_sel).astype(bf16)

    return kernel, nsem


@jax.jit
def pallas_parallel_sum__sliding_block_cached__moe_arch_mod__decode_kernel(
    A_x: jax.Array,
    A_k_cache: jax.Array,
    A_v_cache: jax.Array,
    A_wq: jax.Array,
    A_wo: jax.Array,
    B_x: jax.Array,
    B_w_r: jax.Array,
    B_w_gate: jax.Array,
    B_w_up: jax.Array,
    B_w_down: jax.Array,
):
    del B_x
    B, Sq, D = A_x.shape
    _, HKV, SK, _ = A_k_cache.shape
    F = B_w_gate.shape[1]
    W = min(4096, max(256, SK // 4))
    assert B == 1 and Sq == 1
    kernel, nsem = _make_kernel(D, HKV, SK, W, F)
    hbm = pl.BlockSpec(memory_space=pltpu.MemorySpace.HBM)
    return pl.pallas_call(
        kernel,
        out_shape=jax.ShapeDtypeStruct((B, Sq, D), A_x.dtype),
        in_specs=[hbm] * 9,
        out_specs=pl.BlockSpec(memory_space=pltpu.MemorySpace.VMEM),
        scratch_shapes=[
            pltpu.VMEM((B, Sq, D), bf16),
            pltpu.VMEM((D,), bf16),
            pltpu.VMEM((HKV, W, DH), bf16),
            pltpu.VMEM((HKV, W, DH), bf16),
            pltpu.VMEM((D, HQ * DH), bf16),
            pltpu.VMEM((HQ * DH, D), bf16),
            pltpu.VMEM((D, F), bf16),
            pltpu.VMEM((D, F), bf16),
            pltpu.VMEM((F, D), bf16),
            pltpu.VMEM((HKV, 8, DH), f32),
            pltpu.SemaphoreType.DMA((nsem,)),
        ],
        compiler_params=pltpu.CompilerParams(
            vmem_limit_bytes=64 * 1024 * 1024,
            disable_semaphore_checks=True,
        ),
    )(A_x, A_k_cache, A_v_cache, A_wq, A_wo, B_w_r, B_w_gate, B_w_up, B_w_down)
```

```python
import numpy as np

import jax
import jax.numpy as jnp
import jax.experimental.pallas as pl
import jax.experimental.pallas.tpu as pltpu

HQ, DH = 32, 128
EPS = 1e-5
LANES, SUBLANES = 128, 8
WD_MXU_CHUNKS = (768, 512, 256, 128)
WD_VPU_CHUNKS = (96, 32)

f32, bf16 = jnp.float32, jnp.bfloat16


def _round_bf16(v):
    return v.astype(bf16).astype(f32)


def _make_kernel(D, HKV, SK, W, F):
    rep = HQ // HKV
    gcols = rep * DH
    assert DH == LANES and rep + 1 <= SUBLANES and D % LANES == 0
    chunks = WD_MXU_CHUNKS + WD_VPU_CHUNKS
    n_mxu, n_wd = len(WD_MXU_CHUNKS), len(chunks)
    wd_off = [int(o) for o in np.cumsum((0,) + chunks)]
    v0 = wd_off[n_mxu]
    assert wd_off[-1] == F and F - v0 == LANES
    S_X, S_WR, S_WQ, S_WG, S_WU, S_WD = range(6)
    S_K = S_WD + n_wd
    S_V = S_K + HKV
    S_O = S_V + HKV
    n_sem = S_O + HKV
    scale = np.float32(DH ** -0.5)

    def kernel(x_hbm, k_hbm, v_hbm, wq_hbm, wo_hbm, wr_hbm, wg_hbm, wu_hbm, wd_hbm, o_ref,
               xb, wrb, kb, vb, wqb, wob, wgb, wub, wdb, q_scr, h_scr, sems):
        window = pl.ds(SK - W, W)
        copy = pltpu.make_async_copy
        x_cp = copy(x_hbm, xb, sems.at[S_X])
        wr_cp = copy(wr_hbm, wrb, sems.at[S_WR])
        wq_cp = copy(wq_hbm, wqb, sems.at[S_WQ])
        wg_cp = copy(wg_hbm, wgb, sems.at[S_WG])
        wu_cp = copy(wu_hbm, wub, sems.at[S_WU])

        def wd_cp(i):
            rows = pl.ds(wd_off[i], chunks[i])
            return copy(wd_hbm.at[rows, :], wdb.at[rows, :], sems.at[S_WD + i])

        def k_cp(g):
            return copy(k_hbm.at[0, g, window, :], kb.at[g], sems.at[S_K + g])

        def v_cp(g):
            return copy(v_hbm.at[0, g, window, :], vb.at[g], sems.at[S_V + g])

        def wo_rows(g):
            return pl.ds(pl.multiple_of(g * gcols, gcols), gcols)

        def wo_cp(g):
            return copy(wo_hbm.at[wo_rows(g), :], wob.at[wo_rows(g), :], sems.at[S_O + g])

        wq_cp.start()
        x_cp.start()
        wr_cp.start()
        wg_cp.start()
        wu_cp.start()

        def issue(g, carry):
            k_cp(g).start()
            v_cp(g).start()
            wo_cp(g).start()
            return carry

        jax.lax.fori_loop(0, HKV, issue, 0)
        for i in range(n_wd):
            wd_cp(i).start()

        x_cp.wait()
        wr_cp.wait()
        x = xb[0].astype(f32)
        mu = jnp.mean(x, axis=-1, keepdims=True)
        xc = x - mu
        var = jnp.mean(xc * xc, axis=-1, keepdims=True)
        xn = _round_bf16(xc / jnp.sqrt(var + EPS))
        r = jnp.sum(xn * wrb[...].astype(f32).reshape(1, D), axis=-1, keepdims=True)
        r_sel = jax.nn.sigmoid(_round_bf16(r))
        xn8 = jnp.broadcast_to(xn, (SUBLANES, D)).astype(bf16)

        row = jax.lax.broadcasted_iota(jnp.int32, (SUBLANES, DH), 0)

        wq_cp.wait()
        for g in range(HKV):
            qc = jnp.dot(xn8, wqb[:, g * gcols:(g + 1) * gcols], preferred_element_type=f32)
            qg = qc[:, 0:DH]
            for j in range(1, rep):
                qg = jnp.where(row == j, qc[:, j * DH:(j + 1) * DH], qg)
            q_scr[g] = qg

        wg_cp.wait()
        gate = _round_bf16(jnp.dot(xn8, wgb[...], preferred_element_type=f32))
        wu_cp.wait()
        up = _round_bf16(jnp.dot(xn8, wub[...], preferred_element_type=f32))
        h = (jax.nn.silu(gate) * up).astype(bf16)
        h_tail = h[0:1, v0:F].astype(f32) * r_sel
        h_scr[...] = jnp.broadcast_to(h_tail, (LANES, LANES)).T

        def attend(g, acc):
            k_cp(g).wait()
            q = q_scr[g].astype(bf16)
            s = jax.lax.dot_general(q, kb[g], (((1,), (1,)), ((), ())),
                                    preferred_element_type=f32)
            m = jnp.max(s, axis=-1, keepdims=True)
            p = jnp.exp((s - m) * scale)
            l = jnp.sum(p, axis=-1, keepdims=True)
            v_cp(g).wait()
            o = jnp.dot(p.astype(bf16), vb[g], preferred_element_type=f32) / l
            o = _round_bf16(o)
            lhs = jnp.concatenate([jnp.where(row == j, o, 0.0) for j in range(rep)], axis=1)
            wo_cp(g).wait()
            return acc + jnp.dot(lhs.astype(bf16), wob[wo_rows(g), :], preferred_element_type=f32)

        acc = jax.lax.fori_loop(0, HKV, attend, jnp.zeros((SUBLANES, D), f32))

        y = jnp.zeros((SUBLANES, D), f32)
        for i in range(n_mxu):
            wd_cp(i).wait()
            lo, hi = wd_off[i], wd_off[i + 1]
            y = y + jnp.dot(h[:, lo:hi], wdb[lo:hi, :], preferred_element_type=f32)

        row_d = jax.lax.broadcasted_iota(jnp.int32, (SUBLANES, D), 0)
        rest = jnp.broadcast_to(x + xn + y[0:1] * r_sel, (SUBLANES, D))
        total = jnp.where(row_d == rep, rest, acc)
        parts = [total[:, c:c + LANES] for c in range(0, D, LANES)]

        for i in range(n_mxu, n_wd):
            wd_cp(i).wait()
            for k in range(wd_off[i], wd_off[i + 1], 2 * SUBLANES):
                w = wdb[k:k + 2 * SUBLANES, :].astype(f32)
                h0 = h_scr[k - v0:k - v0 + SUBLANES, :]
                h1 = h_scr[k - v0 + SUBLANES:k - v0 + 2 * SUBLANES, :]
                for j in range(len(parts)):
                    c = j * LANES
                    parts[j] = parts[j] + (w[:SUBLANES, c:c + LANES] * h0 + w[SUBLANES:, c:c + LANES] * h1)
        out = jnp.concatenate([jnp.sum(p, axis=0, keepdims=True) for p in parts], axis=1)
        o_ref[0] = out.astype(o_ref.dtype)

    return kernel, n_sem


@jax.jit
def pallas_parallel_sum__sliding_block_cached__moe_arch_mod__decode_kernel(
    A_x: jax.Array,
    A_k_cache: jax.Array,
    A_v_cache: jax.Array,
    A_wq: jax.Array,
    A_wo: jax.Array,
    B_x: jax.Array,
    B_w_r: jax.Array,
    B_w_gate: jax.Array,
    B_w_up: jax.Array,
    B_w_down: jax.Array,
):
    del B_x
    B, Sq, D = A_x.shape
    _, HKV, SK, _ = A_k_cache.shape
    F = B_w_gate.shape[1]
    W = min(4096, max(256, SK // 4))
    assert B == 1 and Sq == 1
    kernel, n_sem = _make_kernel(D, HKV, SK, W, F)
    hbm = pl.BlockSpec(memory_space=pltpu.MemorySpace.HBM)
    return pl.pallas_call(
        kernel,
        out_shape=jax.ShapeDtypeStruct((B, Sq, D), A_x.dtype),
        in_specs=[hbm] * 9,
        out_specs=pl.BlockSpec(memory_space=pltpu.MemorySpace.VMEM),
        scratch_shapes=[
            pltpu.VMEM((B, Sq, D), bf16),
            pltpu.VMEM((D,), bf16),
            pltpu.VMEM((HKV, W, DH), bf16),
            pltpu.VMEM((HKV, W, DH), bf16),
            pltpu.VMEM((D, HQ * DH), bf16),
            pltpu.VMEM((HQ * DH, D), bf16),
            pltpu.VMEM((D, F), bf16),
            pltpu.VMEM((D, F), bf16),
            pltpu.VMEM((F, D), bf16),
            pltpu.VMEM((HKV, SUBLANES, DH), f32),
            pltpu.VMEM((LANES, LANES), f32),
            pltpu.SemaphoreType.DMA((n_sem,)),
        ],
        compiler_params=pltpu.CompilerParams(
            vmem_limit_bytes=64 * 1024 * 1024,
            disable_semaphore_checks=True,
        ),
    )(A_x, A_k_cache, A_v_cache, A_wq, A_wo, B_w_r, B_w_gate, B_w_up, B_w_down)
```
